```python
import os as _os
_os.environ.setdefault("JAX_PLATFORMS", "cpu")
import jax
import jax.numpy as jnp

def _softmax(x, axis=-1):
    return jax.nn.softmax(x, axis=axis)
def _gelu(x):
    return jax.nn.gelu(x, approximate=True)
def _silu(x):
    return jax.nn.silu(x)
def _sigmoid(x):
    return jax.nn.sigmoid(x)
def _layernorm(x, axis=-1, eps=1e-5):
    m = jnp.mean(x, axis=axis, keepdims=True)
    v = jnp.var(x, axis=axis, keepdims=True)
    return (x - m) / jnp.sqrt(v + eps)
def _scatter_add(tgt, idx, src, axis=0):
    return tgt.at[idx].add(src)
def _segment_sum(src, seg, n):
    return jax.ops.segment_sum(src, seg, n)
class _Rng:
    def __init__(self, key):
        self._k = key
    def _next(self):
        self._k, sub = jax.random.split(self._k)
        return sub
    def normal(self, shape):
        return jax.random.normal(self._next(), shape, dtype=jnp.bfloat16)
    def randint(self, lo, hi, shape):
        return jax.random.randint(self._next(), shape, lo, hi, dtype=jnp.int32)
    def uniform(self, shape, lo=0.0, hi=1.0):
        return jax.random.uniform(self._next(), shape, jnp.bfloat16, lo, hi)
    def permutation(self, n):
        return jax.random.permutation(self._next(), n)


kernel_name = 'gated_mix__mha_block__mixer_s_mlp__prompt'

def setup_inputs():
    _rng = _Rng(jax.random.key(int.from_bytes(__import__("os").urandom(4), "little")))
    _w = (lambda a: (lambda t: t.astype(jnp.bfloat16) if jnp.issubdtype(t.dtype, jnp.floating) else t)(jnp.asarray(a)))
    def _A_setup():
        B, S, D, H = 1, 2048, 512, 32
        return {
            "x": _w((lambda *s: _rng.normal(s) * 0.05)(B, S, D)),
            "wqkv": _w((lambda *s: _rng.normal(s) * 0.8)(D, 3 * D)),
            "wo": _w((lambda *s: _rng.normal(s) * 0.05)(D, D)),
        }
    _A_in = _A_setup()

    def _B_setup():
        B, S, D, F = 1, 2048, 512, 1792
        return {
            "x":  _w((lambda *s: _rng.normal(s) * 0.05)(B, S, D)),
            "w1": _w((lambda *s: _rng.normal(s) * 0.2)(D, D) * (D ** -0.5)),
            "w2": _w((lambda *s: _rng.normal(s) * 0.2)(D, D) * (D ** -0.5)),
            "w3": _w((lambda *s: _rng.normal(s) * 0.2)(D, F) * (D ** -0.5)),
            "w4": _w((lambda *s: _rng.normal(s) * 0.2)(F, D) * (F ** -0.5)),
        }
    _B_in = _B_setup()

    return {
        "A_x": _A_in["x"],
        "A_wqkv": _A_in["wqkv"],
        "A_wo": _A_in["wo"],
        "B_x": _B_in["x"],
        "B_w1": _B_in["w1"],
        "B_w2": _B_in["w2"],
        "B_w3": _B_in["w3"],
        "B_w4": _B_in["w4"],
        "gate_w": _w((lambda *s: _rng.normal(s) * 0.05)(512) * 16.0),
    }

def reference(A_x, A_wqkv, A_wo, B_x, B_w1, B_w2, B_w3, B_w4, gate_w):
    def _A_ref(x, wqkv, wo):
        B, S, D = x.shape
        H = 32
        Dh = D // H
        qkv = (lambda x, *d: x.transpose(*d))((x @ wqkv).reshape(B, S, 3, H, Dh), 2, 0, 3, 1, 4)
        q, k, v = qkv[0], qkv[1], qkv[2]
        scores = jnp.einsum("bhqd,bhkd->bhqk", q, k) * (Dh ** -0.5)
        p = _softmax(scores, axis=-1)
        o = jnp.einsum("bhqk,bhkd->bhqd", p, v)
        return (lambda x, *d: x.transpose(*d))(o, 0, 2, 1, 3).reshape(B, S, D) @ wo

    def _B_ref(x, w1, w2, w3, w4):
        B, S, D = x.shape
        h = _gelu(_layernorm(x, axis=-1) @ w1)
        c = D // 4
        g0 = jnp.pad(h[:, :, 0*c:1*c], ((0, 0), (1, 0), (0, 0)))[:, :S, :]
        g1 = jnp.pad(h[:, :, 1*c:2*c], ((0, 0), (0, 1), (0, 0)))[:, 1:, :]
        g2 = jnp.pad(h[:, :, 2*c:3*c], ((0, 0), (2, 0), (0, 0)))[:, :S, :]
        g3 = jnp.pad(h[:, :, 3*c:   ], ((0, 0), (0, 2), (0, 0)))[:, 2:, :]
        hs = jnp.concatenate([g0, g1, g2, g3], axis=-1) @ w2
        x1 = x + hs
        h2 = _gelu(_layernorm(x1, axis=-1) @ w3) @ w4
        return x1 + h2

    x = A_x
    g = _sigmoid((x * gate_w).sum(-1, keepdims=True))
    a = _A_ref(x, A_wqkv, A_wo)
    b = _B_ref(x, B_w1, B_w2, B_w3, B_w4)
    return g * a + (1 - g) * b
```

```python
import math

import jax
import jax.numpy as jnp
from jax import lax
import jax.experimental.pallas as pl
import jax.experimental.pallas.tpu as pltpu

F32 = jnp.float32
BF16 = jnp.bfloat16

S = 2048
D = 512
H = 32
DH = 16
FF = 1792
LANES = 128
HPB = LANES // DH

TB1 = 512
TB3 = 512
QG = 512
KC = 128
HB = 4
SKEW = 2
FC = 256
PAD = 8

Q_SCALE = (DH ** -0.5) * math.log2(math.e)
SCORE_BOUND = 40.0
V_HI = 2.0 ** 60
V_LO = 2.0 ** -40

TN = (((0,), (0,)), ((), ()))
TNT = (((0,), (1,)), ((), ()))

NB1 = S // TB1
NB3 = S // TB3
SEM_X = 0
SEM_WK = NB1
SEM_WQ = NB1 + 1
SEM_WV = NB1 + 2
SEM_W1 = NB1 + 3
SEM_WO = NB1 + 4
SEM_W2 = NB1 + 5
SEM_W3 = NB1 + 6
SEM_W4 = NB1 + 7
SEM_GW = NB1 + 8
SEM_OUT = NB1 + 9
NSEM = SEM_OUT + NB3


def _dot(a, b):
    return jnp.dot(a, b, preferred_element_type=F32)


def _dg(a, b, dims):
    return lax.dot_general(a, b, dims, preferred_element_type=F32)


def _layernorm(x):
    m = jnp.mean(x, axis=-1, keepdims=True)
    xc = x - m
    v = jnp.mean(xc * xc, axis=-1, keepdims=True)
    return xc * lax.rsqrt(v + 1e-5)


def _gelu(x):
    c = math.sqrt(2.0 / math.pi)
    return 0.5 * x * (1.0 + jnp.tanh(c * (x + 0.044715 * (x * x * x))))


def _kernel(ax_hbm, wqkv_hbm, wo_hbm, w1_hbm, w2_hbm, w3_hbm, w4_hbm, gw_hbm,
            out_hbm,
            ax_ref, wqkv_ref, wo_ref, w1_ref, w2_ref, w3_ref, w4_ref, gw_ref, out_s,
            k_s, qt_s, vt_s, ot_s, h_s, st_s, sem):
    def x_copy(i):
        r0 = pl.multiple_of(i * TB1, TB1)
        return pltpu.make_async_copy(ax_hbm.at[pl.ds(r0, TB1), :], ax_ref.at[pl.ds(r0, TB1), :], sem.at[SEM_X + i])

    def wcol_copy(j, slot):
        return pltpu.make_async_copy(wqkv_hbm.at[:, pl.ds(j * D, D)], wqkv_ref.at[:, pl.ds(j * D, D)], sem.at[slot])

    def out_copy(i):
        r0 = pl.multiple_of(i * TB3, TB3)
        return pltpu.make_async_copy(out_s.at[pl.ds(r0, TB3), :], out_hbm.at[pl.ds(r0, TB3), :], sem.at[SEM_OUT + i])

    early = [wcol_copy(1, SEM_WK), wcol_copy(0, SEM_WQ), wcol_copy(2, SEM_WV),
             pltpu.make_async_copy(w1_hbm, w1_ref, sem.at[SEM_W1])]
    late = [pltpu.make_async_copy(w2_hbm, w2_ref, sem.at[SEM_W2]),
            pltpu.make_async_copy(wo_hbm, wo_ref, sem.at[SEM_WO]),
            pltpu.make_async_copy(w3_hbm, w3_ref, sem.at[SEM_W3]),
            pltpu.make_async_copy(w4_hbm, w4_ref, sem.at[SEM_W4]),
            pltpu.make_async_copy(gw_hbm, gw_ref, sem.at[SEM_GW])]
    x_copy(0).start()
    for c in early:
        c.start()

    h_s[pl.ds(0, PAD), :] = jnp.zeros((PAD, D), F32)
    h_s[pl.ds(PAD + S, PAD), :] = jnp.zeros((PAD, D), F32)
    st_s[...] = jnp.zeros(st_s.shape, F32)
    for c in early:
        c.wait()
    for i in range(1, NB1):
        x_copy(i).start()
    for c in late:
        c.start()

    def proj_body(i, carry):
        r0 = pl.multiple_of(i * TB1, TB1)
        x_copy(i).wait()
        x = ax_ref[pl.ds(r0, TB1), :]
        kb = _dot(x, wqkv_ref[:, pl.ds(D, D)]).astype(BF16)
        k_s[pl.ds(r0, TB1), :] = kb
        qt = (_dg(wqkv_ref[:, pl.ds(0, D)], x, TNT) * Q_SCALE).astype(BF16)
        qt_s[:, pl.ds(r0, TB1)] = qt
        vt = _dg(wqkv_ref[:, pl.ds(2 * D, D)], x, TNT).astype(BF16)
        vt_s[:, pl.ds(r0, TB1)] = vt
        hb = _gelu(_dot(_layernorm(x.astype(F32)).astype(BF16), w1_ref[...]))
        h_s[pl.ds(PAD + r0, TB1), :] = hb.astype(BF16).astype(F32)
        qf = qt.astype(F32)
        qn = jnp.sum((qf * qf).reshape(H, DH, TB1), axis=1)
        qn = jnp.max(qn.reshape(H // 8, 8, TB1), axis=0)
        qm = qn[:, 0:LANES]
        for j in range(1, TB1 // LANES):
            qm = jnp.maximum(qm, qn[:, j * LANES:(j + 1) * LANES])
        kf = kb.astype(F32)
        kk = kf * kf
        km = None
        for j in range(D // LANES):
            y = kk[:, j * LANES:(j + 1) * LANES]
            for sh in (1, 2, 4, 8):
                y = y + pltpu.roll(y, sh, 1)
            y = jnp.max(y.reshape(TB1 // 8, 8, LANES), axis=0)
            km = y if km is None else jnp.maximum(km, y)
        vf = jnp.abs(vt.astype(F32))
        vm = jnp.max(vf.reshape(D // 8, 8, TB1), axis=0)
        vmm = vm[:, 0:LANES]
        for j in range(1, TB1 // LANES):
            vmm = jnp.maximum(vmm, vm[:, j * LANES:(j + 1) * LANES])
        st_s[0] = jnp.maximum(st_s[0], qm)
        st_s[1] = jnp.maximum(st_s[1], km)
        st_s[2] = jnp.maximum(st_s[2], vmm)
        return carry

    lax.fori_loop(0, NB1, proj_body, 0)

    q2 = jnp.max(st_s[0])
    k2 = jnp.max(st_s[1])
    vmax = jnp.max(st_s[2])
    safe = jnp.logical_and(
        q2 * k2 * 1.01 <= SCORE_BOUND * SCORE_BOUND,
        jnp.logical_and(vmax <= V_HI, vmax >= V_LO))

    nq = S // QG
    nc = S // KC

    def head_weights(h, q0, rows):
        row0 = pl.multiple_of((h // HPB) * LANES, LANES)
        w = qt_s[pl.ds(row0, LANES), pl.ds(q0, QG)]
        w = jnp.where((rows // DH) == (h % HPB), w, jnp.zeros_like(w))
        return row0, w

    @pl.when(safe)
    def _():
        def body(it, carry):
            rows = lax.broadcasted_iota(jnp.int32, (LANES, QG), 0)
            segs = {}

            def seg(hb, qg):
                if (hb, qg) not in segs:
                    h = it * HB + hb
                    row0, w = head_weights(h, qg * QG, rows)
                    segs[(hb, qg)] = dict(
                        row0=row0, w=w, vrow=pl.multiple_of(h * DH, DH),
                        acc=jnp.zeros((DH, QG), F32), l=jnp.zeros((8, QG), F32))
                return segs[(hb, qg)]

            def qk(hb, qg, kc):
                e = seg(hb, qg)
                return _dot(k_s[pl.ds(kc * KC, KC), pl.ds(e["row0"], LANES)], e["w"])

            def pv(hb, qg, kc, s):
                e = seg(hb, qg)
                p = jnp.exp2(s)
                e["l"] = e["l"] + jnp.sum(p.reshape(KC // 8, 8, QG), axis=0)
                e["acc"] = e["acc"] + _dot(vt_s[pl.ds(e["vrow"], DH), pl.ds(kc * KC, KC)], p.astype(BF16))
                if kc == nc - 1:
                    lt = jnp.sum(e["l"], axis=0, keepdims=True)
                    ot_s[pl.ds(e["vrow"], DH), pl.ds(qg * QG, QG)] = (e["acc"] / lt).astype(BF16)

            pend = []
            for hb in range(HB):
                for qg in range(nq):
                    for kc in range(nc):
                        pend.append((hb, qg, kc, qk(hb, qg, kc)))
                        if len(pend) > SKEW:
                            pv(*pend.pop(0))
            while pend:
                pv(*pend.pop(0))
            return carry

        lax.fori_loop(0, H // HB, body, 0)

    @pl.when(jnp.logical_not(safe))
    def _():
        def body(it, carry):
            h = it // nq
            q0 = pl.multiple_of((it % nq) * QG, QG)
            rows = lax.broadcasted_iota(jnp.int32, (LANES, QG), 0)
            row0, w = head_weights(h, q0, rows)
            vrow = pl.multiple_of(h * DH, DH)
            s = _dot(k_s[:, pl.ds(row0, LANES)], w)
            m = jnp.max(s, axis=0, keepdims=True)
            p = jnp.exp2(s - m)
            lt = jnp.sum(p, axis=0, keepdims=True)
            acc = _dot(vt_s[pl.ds(vrow, DH), :], p.astype(BF16))
            ot_s[pl.ds(vrow, DH), pl.ds(q0, QG)] = (acc / lt).astype(BF16)
            return carry

        lax.fori_loop(0, H * nq, body, 0)

    for c in late:
        c.wait()

    def out_body(i, carry):
        r0 = pl.multiple_of(i * TB3, TB3)
        parts = []
        for gi, sh in enumerate((-1, 1, -2, 2)):
            win = h_s[pl.ds(r0, TB3 + 2 * PAD), pl.ds(gi * LANES, LANES)]
            parts.append(win[PAD + sh:PAD + sh + TB3, :])
        hs = jnp.concatenate(parts, axis=1).astype(BF16)
        xf = ax_ref[pl.ds(r0, TB3), :].astype(F32)
        x1 = xf + _dot(hs, w2_ref[...])
        a = _dg(ot_s[:, pl.ds(r0, TB3)], wo_ref[...], TN)
        ln = _layernorm(x1).astype(BF16)
        y = x1
        nf = FF // FC
        t_next = _dot(ln, w3_ref[:, pl.ds(0, FC)])
        for c in range(nf):
            t = t_next
            if c + 1 < nf:
                t_next = _dot(ln, w3_ref[:, pl.ds((c + 1) * FC, FC)])
            y = y + _dot(_gelu(t).astype(BF16), w4_ref[pl.ds(c * FC, FC), :])
        xg = xf * gw_ref[...].astype(F32).reshape(1, D)
        g = jax.nn.sigmoid(jnp.sum(xg, axis=-1, keepdims=True))
        out_s[pl.ds(r0, TB3), :] = (g * a + (1.0 - g) * y).astype(out_s.dtype)
        out_copy(i).start()
        return carry

    lax.fori_loop(0, NB3, out_body, 0)
    for i in range(NB3):
        out_copy(i).wait()


@jax.jit
def pallas_gated_mix__mha_block__mixer_s_mlp__prompt_kernel(
    A_x: jax.Array,
    A_wqkv: jax.Array,
    A_wo: jax.Array,
    B_x: jax.Array,
    B_w1: jax.Array,
    B_w2: jax.Array,
    B_w3: jax.Array,
    B_w4: jax.Array,
    gate_w: jax.Array,
):
    del B_x
    hbm = pl.BlockSpec(memory_space=pl.ANY)
    out = pl.pallas_call(
        _kernel,
        out_shape=jax.ShapeDtypeStruct((S, D), BF16),
        in_specs=[hbm] * 8,
        out_specs=hbm,
        scratch_shapes=[
            pltpu.VMEM((S, D), BF16),
            pltpu.VMEM((D, 3 * D), BF16),
            pltpu.VMEM((D, D), BF16),
            pltpu.VMEM((D, D), BF16),
            pltpu.VMEM((D, D), BF16),
            pltpu.VMEM((D, FF), BF16),
            pltpu.VMEM((FF, D), BF16),
            pltpu.VMEM((D,), BF16),
            pltpu.VMEM((S, D), BF16),
            pltpu.VMEM((S, D), BF16),
            pltpu.VMEM((D, S), BF16),
            pltpu.VMEM((D, S), BF16),
            pltpu.VMEM((D, S), BF16),
            pltpu.VMEM((S + 2 * PAD, D), F32),
            pltpu.VMEM((3, 8, LANES), F32),
            pltpu.SemaphoreType.DMA((NSEM,)),
        ],
        compiler_params=pltpu.CompilerParams(vmem_limit_bytes=100 * 1024 * 1024),
    )(A_x.reshape(S, D), A_wqkv, A_wo, B_w1, B_w2, B_w3, B_w4, gate_w)
    return out.reshape(1, S, D)
```
